```python
import os as _os
_os.environ.setdefault("JAX_PLATFORMS", "cpu")
import jax
import jax.numpy as jnp

def _softmax(x, axis=-1):
    return jax.nn.softmax(x, axis=axis)
def _gelu(x):
    return jax.nn.gelu(x, approximate=True)
def _silu(x):
    return jax.nn.silu(x)
def _sigmoid(x):
    return jax.nn.sigmoid(x)
def _layernorm(x, axis=-1, eps=1e-5):
    m = jnp.mean(x, axis=axis, keepdims=True)
    v = jnp.var(x, axis=axis, keepdims=True)
    return (x - m) / jnp.sqrt(v + eps)
def _scatter_add(tgt, idx, src, axis=0):
    return tgt.at[idx].add(src)
def _segment_sum(src, seg, n):
    return jax.ops.segment_sum(src, seg, n)
class _Rng:
    def __init__(self, key):
        self._k = key
    def _next(self):
        self._k, sub = jax.random.split(self._k)
        return sub
    def normal(self, shape):
        return jax.random.normal(self._next(), shape, dtype=jnp.bfloat16)
    def randint(self, lo, hi, shape):
        return jax.random.randint(self._next(), shape, lo, hi, dtype=jnp.int32)
    def uniform(self, shape, lo=0.0, hi=1.0):
        return jax.random.uniform(self._next(), shape, jnp.bfloat16, lo, hi)
    def permutation(self, n):
        return jax.random.permutation(self._next(), n)


kernel_name = 'sequential_preLN__sliding_local_dilated__dense_activation_relu__prompt'

def setup_inputs():
    _rng = _Rng(jax.random.key(int.from_bytes(__import__("os").urandom(4), "little")))
    _w = (lambda a: (lambda t: t.astype(jnp.bfloat16) if jnp.issubdtype(t.dtype, jnp.floating) else t)(jnp.asarray(a)))
    def _A_setup():
        B, S, D = 1, 2048, 1024
        return {
            "x": _w((lambda *s: _rng.normal(s) * 0.05)(B, S, D)),
            "wqkv": _w((lambda *s: _rng.normal(s) * 0.05)(D, 3 * D)),
            "wo": _w((lambda *s: _rng.normal(s) * 0.05)(D, D)),
        }
    _A_in = _A_setup()

    def _B_setup():
        B, S, D, Dff = 1, 2048, 1024, 3584
        return {
            "x": _w((lambda *s: _rng.normal(s) * 0.05)(B, S, D)),
            "w1": _w((lambda *s: _rng.normal(s) * 0.05)(D, Dff)),
            "w2": _w((lambda *s: _rng.normal(s) * 0.05)(Dff, D)),
        }
    _B_in = _B_setup()

    return {
        "A_x": _A_in["x"],
        "A_wqkv": _A_in["wqkv"],
        "A_wo": _A_in["wo"],
        "B_x": _B_in["x"],
        "B_w1": _B_in["w1"],
        "B_w2": _B_in["w2"],
    }

def reference(A_x, A_wqkv, A_wo, B_x, B_w1, B_w2):
    def _A_ref(x, wqkv, wo):
        B, S, D = x.shape
        H = 32; Dh = D // H
        W, dil = 8, 2
        qkv = (lambda x, *d: x.transpose(*d))((x @ wqkv).reshape(B, S, 3, H, Dh), 2, 0, 3, 1, 4)
        q, k, v = qkv[0], qkv[1], qkv[2]
        scale = Dh ** -0.5
        pos = jnp.arange(S)
        off = jnp.arange(W) * dil
        idx = pos[:, None] - off[None, :]
        mask = idx >= 0
        idx_c = jnp.where(mask, idx, 0).reshape(-1)
        kg = k[:, :, idx_c, :].reshape(B, H, S, W, Dh)
        vg = v[:, :, idx_c, :].reshape(B, H, S, W, Dh)
        logits = jnp.einsum("bhsd,bhswd->bhsw", q, kg) * scale
        logits = jnp.where(mask[None, None, :, :], logits, -1e9)
        attn = _softmax(logits, axis=-1)
        o = jnp.einsum("bhsw,bhswd->bhsd", attn, vg)
        return (lambda x, *d: x.transpose(*d))(o, 0, 2, 1, 3).reshape(B, S, D) @ wo

    def _B_ref(x, w1, w2):
        h = jnp.einsum("bsd,df->bsf", x, w1)
        zero = jnp.zeros_like(h)
        h = jnp.maximum(h, zero)
        return jnp.einsum("bsf,fd->bsd", h, w2)

    x = A_x
    h = x + _A_ref(_layernorm(x, axis=-1), A_wqkv, A_wo)
    h2 = h + _B_ref(_layernorm(h, axis=-1), B_w1, B_w2)
    return h2
```

```python
import functools

import jax
import jax.numpy as jnp
import numpy as np
from jax.experimental import pallas as pl
from jax.experimental.pallas import tpu as pltpu

BF = jnp.bfloat16
F32 = jnp.float32
U32 = jnp.uint32
I32 = jnp.int32

S, D, FF = 2048, 1024, 3584
H, DH, W, DIL = 32, 32, 8, 2
T = 256
NT = S // T
TW = T // 2
G = D // 128
EPS = 1e-5
SCALE = DH ** -0.5

PMODE = "sparse2"
EMODE = "sparse2"
ESPLIT = int("2")
HBF = int("1")
LNROWS = int("8")
RA = int("1")
RB = int("1")
OSPLIT = int("3")
PJ = int("3")
EJ = int("7")
assert all(6 * PJ + EJ * (i + 1) >= 8 * (i + 2) for i in range(7)) and 6 * PJ >= 8
CH = int("4")
PF = int("2")
XAT = int("4")


def _ln(x):
    m = jnp.mean(x, axis=-1, keepdims=True)
    xc = x - m
    v = jnp.mean(xc * xc, axis=-1, keepdims=True)
    return xc * jax.lax.rsqrt(v + EPS)


def _unp(w, par):
    return pltpu.unpack_elementwise(w, index=par, packed_dtype=BF, unpacked_dtype=F32)


def _rs8(p):
    sub = jax.lax.broadcasted_iota(I32, (8, 128), 0)

    def comb(a, b, sh):
        m = (sub & sh) == 0
        t = jnp.where(m, a, b)
        u = jnp.where(m, b, a)
        return t + jnp.take_along_axis(u, sub ^ sh, axis=0)

    s1 = [comb(p[i], p[i + 4], 4) for i in range(4)]
    s2 = [comb(s1[i], s1[i + 2], 2) for i in range(2)]
    return comb(s2[0], s2[1], 1)


def _softmax_rows(part, valid):
    l = _rs8(part) * SCALE
    l = jnp.where(valid, l, -1e9)
    m = jnp.max(l, axis=0, keepdims=True)
    e = jnp.exp(l - m)
    a = e / jnp.sum(e, axis=0, keepdims=True)
    return [jnp.broadcast_to(a[w:w + 1], (8, 128)) for w in range(W)]


def _attention_steps(j0, nj, qkv_ref, kp_ref, vp_ref, o_ref, mode):
    lane8 = jax.lax.broadcasted_iota(I32, (8, 128), 1)
    sub8 = jax.lax.broadcasted_iota(I32, (8, 128), 0)
    never = (lane8 + j0) < 0

    def job(n):
        j = j0 + n
        t = jnp.minimum(j // G, NT - 1)
        return t, jnp.minimum(j // G, NT), j % G

    def tr(n, part):
        t, _, g = job(n)
        return qkv_ref[t, :, pl.ds(pl.multiple_of((part * G + g) * 128, 128), 128)].T

    def shifted(cur, prv, w):
        if w == 0:
            return cur
        return pltpu.roll(jnp.where(lane8 >= 128 - w, prv, cur), w, 1)

    def link(x, dep):
        if dep is None:
            return x
        return jnp.where(never, jax.lax.bitcast_convert_type(dep, x.dtype), x)

    def put(n, words):
        _, slot, g = job(n)
        o_ref[pl.ds(pl.multiple_of(slot * TW, TW), TW), pl.ds(pl.multiple_of(g * 128, 128), 128)] = words.T

    qT_n, kT_n, vT_n = tr(0, 0), tr(0, 1), tr(0, 2)
    prev = None
    pend = None
    for n in range(nj):
        t, _, g = job(n)
        valid = (lane8 + t * TW) >= sub8
        qT, kT, vT = qT_n, kT_n, vT_n
        kp = kp_ref[g]
        vp = vp_ref[g]
        kp_ref[g] = kT
        vp_ref[g] = vT
        words = []
        for h in range(4):
            sl = [slice(32 * h + 8 * j, 32 * h + 8 * j + 8) for j in range(4)]
            if mode == "dense":
                q = [[_unp(qT[sl[j]], par) for j in range(4)] for par in range(2)]
                part = [[], []]
                for w in range(W):
                    kw = [shifted(kT[sl[j]], kp[sl[j]], w) for j in range(4)]
                    kw[0] = link(kw[0], prev)
                    for par in range(2):
                        k = [_unp(kw[j], par) for j in range(4)]
                        part[par].append((q[par][0] * k[0] + q[par][1] * k[1]) + (q[par][2] * k[2] + q[par][3] * k[3]))
                    prev = jnp.maximum(part[0][w], part[1][w])
                att = [_softmax_rows(part[par], valid) for par in range(2)]
                prev = None
                for j in range(4):
                    vw = [shifted(vT[sl[j]], vp[sl[j]], w) for w in range(W)]
                    vw[0] = link(vw[0], prev)
                    acc = []
                    for par in range(2):
                        a = None
                        for w in range(W):
                            c = att[par][w] * _unp(vw[w], par)
                            a = c if a is None else a + c
                        acc.append(a)
                    prev = pltpu.pack_elementwise(acc, packed_dtype=BF)
                    words.append(prev)
            else:
                kws = [[shifted(kT[sl[j]], kp[sl[j]], w) for j in range(4)] for w in range(W)]
                att = []
                for par in range(2):
                    q = [_unp(qT[sl[j]], par) for j in range(4)]
                    part = []
                    for w in range(W):
                        k = [_unp(kws[w][j], par) for j in range(4)]
                        k[0] = link(k[0], prev)
                        part.append((q[0] * k[0] + q[1] * k[1]) + (q[2] * k[2] + q[3] * k[3]))
                        prev = part[-1]
                    att.append(_softmax_rows(part, valid))
                    prev = att[-1][0] if mode == "sparse2" else prev
                for j in range(4):
                    vw = [shifted(vT[sl[j]], vp[sl[j]], w) for w in range(W)]
                    acc = []
                    for par in range(2):
                        a = None
                        for w in range(W):
                            v = _unp(vw[w], par)
                            if w == 0:
                                v = link(v, prev)
                            c = att[par][w] * v
                            a = c if a is None else a + c
                        acc.append(a)
                        prev = a
                    words.append(pltpu.pack_elementwise(acc, packed_dtype=BF))
            if h == 0 and pend is not None:
                put(n - 1, pend)
                pend = None
            if n + 1 < nj:
                if h == 1:
                    qT_n = tr(n + 1, 0)
                elif h == 2:
                    kT_n = tr(n + 1, 1)
                elif h == 3:
                    vT_n = tr(n + 1, 2)
            yield
        pend = jnp.concatenate(words, axis=0)
    put(nj - 1, pend)


def _ln_steps(t, x_ref, xn_ref, rows=16):
    for r in range(0, T, rows):
        r0 = pl.multiple_of(t * T + r, rows)
        xn_ref[r:r + rows, :] = _ln(x_ref[pl.ds(r0, rows), :].astype(F32)).astype(BF)
        yield


def _interleave(*gens, ratio=None):
    gens = list(gens)
    ratio = ratio or [1] * len(gens)
    alive = [True] * len(gens)
    while any(alive):
        for i, gen in enumerate(gens):
            for _ in range(ratio[i]):
                if alive[i]:
                    try:
                        next(gen)
                    except StopIteration:
                        alive[i] = False


def _wt(ref, j):
    return pltpu.bitcast(ref.bitcast(U32)[j], BF)


def _kernel(x_hbm, wqkv_hbm, wo_hbm, w1_hbm, w2_hbm, out_hbm,
            x_v, wqkv_v, wo_v, w1_v, w2_v, xn_v, qkv_v, kp_v, vp_v, o_v, out_v,
            sem_x, sem_q, sem_w, sem_o):
    NQ = 3 * D // 128

    def x_cp(i):
        r = pl.ds(pl.multiple_of(i * T, T), T)
        return pltpu.make_async_copy(x_hbm.at[r], x_v.at[r], sem_x.at[i])

    def wq_cp(c):
        return pltpu.make_async_copy(wqkv_hbm.at[:, pl.ds(pl.multiple_of(c * 128, 128), 128)], wqkv_v.at[c], sem_q.at[c])

    def start_cols(w_hbm, w_v, sem):
        for j in range(w_v.shape[0]):
            pltpu.make_async_copy(w_hbm.at[:, j * 128:(j + 1) * 128], w_v.at[j], sem).start()

    def start_rest(s, nsteps):
        for n, (w_hbm, w_v) in enumerate(((wo_hbm, wo_v), (w1_hbm, w1_v), (w2_hbm, w2_v))):
            nt = w_v.shape[0]
            per = -(-nt // nsteps)
            for k in range(per):
                j = s * per + k

                @pl.when(j < nt)
                def _():
                    pltpu.make_async_copy(w_hbm.at[:, pl.ds(pl.multiple_of(j * 128, 128), 128)], w_v.at[j], sem_w.at[n]).start()

    def wait_rest():
        for n, w_v in enumerate((wo_v, w1_v, w2_v)):
            pltpu.make_async_copy(w_v, w_v, sem_w.at[n]).wait()

    def wcat(w_v, cols=None):
        cols = range(w_v.shape[0]) if cols is None else cols
        return jnp.concatenate([_wt(w_v, j) for j in cols], axis=1)

    x_cp(0).start()
    x_cp(1).start()
    for c in range(4):
        wq_cp(c).start()
    xn_an = pltpu.annotate(xn_v, no_hazard_no_deps=True)

    kp_v[...] = jnp.zeros_like(kp_v)
    vp_v[...] = jnp.zeros_like(vp_v)

    with jax.named_scope("P0"):
        x_cp(0).wait()
        for _ in _ln_steps(0, x_v, xn_v.at[0], rows=64):
            pass
        x_cp(1).wait()
        for _ in _ln_steps(1, x_v, xn_v.at[1], rows=64):
            pass

        def qkv01(c):
            xn2 = jnp.concatenate([xn_v[0], xn_v[1]], axis=0)
            r = pltpu.bitcast(jnp.dot(xn2, _wt(wqkv_v, c), preferred_element_type=F32).astype(BF), U32)
            col = pl.ds(pl.multiple_of(c * 128, 128), 128)
            qkv_v[0, :, col] = r[:TW]
            qkv_v[1, :, col] = r[TW:]

        def p0a(it, _):
            for j in range(2):
                wq_cp(2 * it + j).wait()
            for j in range(3):
                wq_cp(4 + 3 * it + j).start()

            @pl.when(it == 2)
            def _():
                x_cp(2).start()
            for j in range(2):
                qkv01(2 * it + j)
            return 0

        def p0b(it, _):
            for j in range(6):
                wq_cp(6 + 6 * it + j).wait()

            @pl.when(it == 0)
            def _():
                x_cp(2).wait()
                for j in range(13, 19):
                    wq_cp(j).start()

            @pl.when(it == 1)
            def _():
                for j in range(19, NQ):
                    wq_cp(j).start()
                for i in range(3, NT):
                    x_cp(i).start()

            for j in range(6):
                qkv01(6 + 6 * it + j)
            for r in range(0, 96, 16):
                r0 = pl.multiple_of(80 * it + r, 16)
                xn_an[2, pl.ds(r0, 16), :] = _ln(x_v[pl.ds(2 * T + r0, 16), :].astype(F32)).astype(BF)
            return 0

        jax.lax.fori_loop(0, 3, p0a, 0)
        jax.lax.fori_loop(0, 3, p0b, 0)

    def stage_b(xn_ref, qkv_ref):
        xn = xn_ref[...]
        for c in range(NQ):
            r = jnp.dot(xn, _wt(wqkv_v, c), preferred_element_type=F32).astype(BF)
            qkv_ref[:, c * 128:(c + 1) * 128] = pltpu.bitcast(r, U32)

    qkv_an = pltpu.annotate(qkv_v, no_hazard_no_deps=True)

    def pstep(s, _):
        @pl.when(s + 3 < NT)
        def _():
            x_cp(s + 3).wait()
        start_rest(s, 4)
        stage_b(xn_an.at[(s + 2) % 3], qkv_an.at[s + 2])
        _interleave(_attention_steps(s * PJ, PJ, qkv_an, kp_v, vp_v, o_v, PMODE),
                    _ln_steps(jnp.minimum(s + 3, NT - 1), x_v, xn_an.at[s % 3], rows=LNROWS), ratio=[RA, RB])
        return 0

    with jax.named_scope("PL"):
        jax.lax.fori_loop(0, NT - 2, pstep, 0)
    with jax.named_scope("BR"):
        wait_rest()

    def out_copy(i, slot, a=None):
        if a is None:
            return pltpu.make_async_copy(out_v.at[slot], out_hbm.at[pl.ds(pl.multiple_of(i * T, T), T)], sem_o.at[slot])
        if OSPLIT == 2:
            HT = T // 2
            return pltpu.make_async_copy(out_v.at[slot, pl.ds(a * HT, HT)], out_hbm.at[pl.ds(pl.multiple_of(i * T + a * HT, HT), HT)], sem_o.at[slot])
        return pltpu.make_async_copy(out_v.at[slot, :, pl.ds(a * 512, 512)], out_hbm.at[pl.ds(pl.multiple_of(i * T, T), T), pl.ds(a * 512, 512)], sem_o.at[slot])

    def estep(i, _):
        slot = i % 2

        @pl.when(i >= 2)
        def _():
            out_copy(i - 2, slot).wait()
        HT = T // ESPLIT
        hs, hns = [], []
        for a in range(ESPLIT):
            r0 = pl.multiple_of(i * T + a * HT, HT)
            rw = pl.multiple_of(i * TW + a * (HT // 2), HT // 2)
            o = pltpu.bitcast(o_v[pl.ds(rw, HT // 2), :], BF)
            att = jnp.dot(o, wcat(wo_v), preferred_element_type=F32)
            if HBF:
                att = att.astype(BF).astype(F32)
            h = x_v[pl.ds(r0, HT), :].astype(F32) + att
            if HBF:
                h = h.astype(BF).astype(F32)
            hs.append(h)
        for a in range(ESPLIT):
            hns.append(jnp.concatenate([_ln(hs[a][r:r + 16]).astype(BF) for r in range(0, HT, 16)], axis=0))
        hid = jnp.concatenate(
            [jnp.maximum(jnp.dot(hns[a], wcat(w1_v), preferred_element_type=F32), 0.0).astype(BF) for a in range(ESPLIT)], axis=0)
        if OSPLIT == 1:
            out = jnp.concatenate(hs, axis=0) + jnp.dot(hid, wcat(w2_v), preferred_element_type=F32)
            out_v[slot] = out.astype(BF)
            out_copy(i, slot).start()
        elif OSPLIT == 2:
            for a in range(2):
                out = hs[a] + jnp.dot(hid[a * HT:(a + 1) * HT], wcat(w2_v), preferred_element_type=F32)
                out_v[slot, a * HT:(a + 1) * HT, :] = out.astype(BF)
                out_copy(i, slot, a).start()
        else:
            hcat = jnp.concatenate(hs, axis=0)
            for a in range(2):
                cs = slice(a * 512, (a + 1) * 512)
                out = hcat[:, cs] + jnp.dot(hid, wcat(w2_v, range(4 * a, 4 * a + 4)), preferred_element_type=F32)
                out_v[slot, :, cs] = out.astype(BF)
                out_copy(i, slot, a).start()
        for _ in _attention_steps((NT - 2) * PJ + i * EJ, EJ, qkv_v, kp_v, vp_v, o_v, EMODE):
            pass
        return 0

    with jax.named_scope("EL"):
        jax.lax.fori_loop(0, NT, estep, 0)
    with jax.named_scope("FIN"):
        out_copy(NT - 2, (NT - 2) % 2).wait()
        out_copy(NT - 1, (NT - 1) % 2).wait()


@jax.jit
def pallas_sequential_preLN__sliding_local_dilated__dense_activation_relu__prompt_kernel(A_x, A_wqkv, A_wo, B_x, B_w1, B_w2):
    del B_x
    x2 = A_x.reshape(S, D)
    out = pl.pallas_call(
        _kernel,
        out_shape=jax.ShapeDtypeStruct((S, D), BF),
        in_specs=[pl.BlockSpec(memory_space=pl.ANY)] * 5,
        out_specs=pl.BlockSpec(memory_space=pl.ANY),
        scratch_shapes=[
            pltpu.VMEM((S, D), BF),
            pltpu.VMEM((3 * D // 128, D, 128), BF),
            pltpu.VMEM((D // 128, D, 128), BF),
            pltpu.VMEM((FF // 128, D, 128), BF),
            pltpu.VMEM((D // 128, FF, 128), BF),
            pltpu.VMEM((3, T, D), BF),
            pltpu.VMEM((NT, TW, 3 * D), U32),
            pltpu.VMEM((G, 128, 128), U32),
            pltpu.VMEM((G, 128, 128), U32),
            pltpu.VMEM(((NT + 1) * TW, D), U32),
            pltpu.VMEM((2, T, D), BF),
            pltpu.SemaphoreType.DMA((NT,)),
            pltpu.SemaphoreType.DMA((3 * D // 128,)),
            pltpu.SemaphoreType.DMA((3,)),
            pltpu.SemaphoreType.DMA((2,)),
        ],
        compiler_params=pltpu.CompilerParams(vmem_limit_bytes=100 * 1024 * 1024),
        name="fused",
    )(x2, A_wqkv, A_wo, B_w1, B_w2)
    return out.reshape(1, S, D)
```

```python
import jax
import jax.numpy as jnp
from jax.experimental import pallas as pl
from jax.experimental.pallas import tpu as pltpu

BF = jnp.bfloat16
F32 = jnp.float32
U32 = jnp.uint32
I32 = jnp.int32

S, D, FF = 2048, 1024, 3584
DH, W = 32, 8
EPS = 1e-5
SCALE = DH ** -0.5

T = 256
NT = S // T
TW = T // 2
G = D // 128
CW = 256
PJ = 3
EJ = 7


def _ln(x):
    m = jnp.mean(x, axis=-1, keepdims=True)
    xc = x - m
    v = jnp.mean(xc * xc, axis=-1, keepdims=True)
    return xc * jax.lax.rsqrt(v + EPS)


def _unpack(w, half):
    bits = (w << 16) if half == 0 else (w & jnp.uint32(0xFFFF0000))
    return jax.lax.bitcast_convert_type(bits, F32)


def _pack(lo, hi):
    lo = jax.lax.bitcast_convert_type(lo, U32) + jnp.uint32(0x8000)
    hi = jax.lax.bitcast_convert_type(hi, U32) + jnp.uint32(0x8000)
    return (lo >> 16) | (hi & jnp.uint32(0xFFFF0000))


def _sum_rows(p):
    sub = jax.lax.broadcasted_iota(I32, (8, 128), 0)

    def merge(a, b, sh):
        m = (sub & sh) == 0
        return jnp.where(m, a, b) + jnp.take_along_axis(jnp.where(m, b, a), sub ^ sh, axis=0)

    s1 = [merge(p[i], p[i + 4], 4) for i in range(4)]
    s2 = [merge(s1[i], s1[i + 2], 2) for i in range(2)]
    return merge(s2[0], s2[1], 1)


def _softmax_rows(part, valid):
    l = _sum_rows(part) * SCALE
    l = jnp.where(valid, l, -1e9)
    m = jnp.max(l, axis=0, keepdims=True)
    e = jnp.exp(l - m)
    a = e / jnp.sum(e, axis=0, keepdims=True)
    return [jnp.broadcast_to(a[w:w + 1], (8, 128)) for w in range(W)]


def _attention_steps(j0, nj, jend, tbase, qkv_ref, kp_ref, vp_ref, o_ref):
    lane8 = jax.lax.broadcasted_iota(I32, (8, 128), 1)
    sub8 = jax.lax.broadcasted_iota(I32, (8, 128), 0)
    never = (lane8 + j0) < 0

    def chain(x, dep):
        if dep is None:
            return x
        return jnp.where(never, jax.lax.bitcast_convert_type(dep, x.dtype), x)

    def job(n):
        j = j0 + n
        jc = jnp.minimum(j, jend - 1)
        return jc // G, jnp.where(j < jend, j // G, NT), jc % G

    def load_t(n, part):
        t, _, g = job(n)
        rows = pl.ds(pl.multiple_of((t - tbase) * TW, TW), TW)
        return qkv_ref[rows, pl.ds(pl.multiple_of((part * G + g) * 128, 128), 128)].T

    def store_t(n, words):
        _, slot, g = job(n)
        rows = pl.ds(pl.multiple_of(slot * TW, TW), TW)
        o_ref[rows, pl.ds(pl.multiple_of(g * 128, 128), 128)] = words.T

    def shifted(cur, prv, w):
        if w == 0:
            return cur
        return pltpu.roll(jnp.where(lane8 >= 128 - w, prv, cur), w, 1)

    q_nxt, k_nxt, v_nxt = load_t(0, 0), load_t(0, 1), load_t(0, 2)
    prev = None
    pend = None
    for n in range(nj):
        t, _, g = job(n)
        valid = (lane8 + t * TW) >= sub8
        qT, kT, vT = q_nxt, k_nxt, v_nxt
        kp = kp_ref[g]
        vp = vp_ref[g]
        kp_ref[g] = kT
        vp_ref[g] = vT
        words = []
        for h in range(4):
            sl = [slice(32 * h + 8 * j, 32 * h + 8 * j + 8) for j in range(4)]
            kws = [[shifted(kT[sl[j]], kp[sl[j]], w) for j in range(4)] for w in range(W)]
            att = []
            for half in range(2):
                q = [_unpack(qT[sl[j]], half) for j in range(4)]
                part = []
                for w in range(W):
                    k = [_unpack(kws[w][j], half) for j in range(4)]
                    k[0] = chain(k[0], prev)
                    prev = (q[0] * k[0] + q[1] * k[1]) + (q[2] * k[2] + q[3] * k[3])
                    part.append(prev)
                att.append(_softmax_rows(part, valid))
                prev = att[-1][0]
            for j in range(4):
                vw = [shifted(vT[sl[j]], vp[sl[j]], w) for w in range(W)]
                acc = []
                for half in range(2):
                    a = att[half][0] * chain(_unpack(vw[0], half), prev)
                    for w in range(1, W):
                        a = a + att[half][w] * _unpack(vw[w], half)
                    acc.append(a)
                    prev = a
                words.append(_pack(*acc))
            if h == 0 and pend is not None:
                store_t(n - 1, pend)
                pend = None
            if n + 1 < nj:
                if h == 1:
                    q_nxt = load_t(n + 1, 0)
                elif h == 2:
                    k_nxt = load_t(n + 1, 1)
                elif h == 3:
                    v_nxt = load_t(n + 1, 2)
            yield
        pend = jnp.concatenate(words, axis=0)
    store_t(nj - 1, pend)


def _rows(ref, r0, n):
    w = ref[pl.ds(pl.multiple_of(r0 // 2, n // 2), n // 2), :]
    return pltpu.bitcast(w, BF).astype(F32)


def _ln_steps(t, x_ref, xn_ref, rows):
    blk = max(rows, 16)
    for r in range(0, T, blk):
        x = _rows(x_ref, t * T + r, blk)
        ys = []
        for q in range(0, blk, rows):
            ys.append(_ln(x[q:q + rows]))
            if q + rows < blk:
                yield
        y = ys[0] if len(ys) == 1 else jnp.concatenate(ys, axis=0)
        xn_ref[r // 2:(r + blk) // 2, :] = pltpu.bitcast(y.astype(BF), U32)
        yield


def _drain(gen):
    for _ in gen:
        pass


def _interleave(*gens):
    alive = list(gens)
    while alive:
        for gen in list(alive):
            if next(gen, alive) is alive:
                alive.remove(gen)


def _kernel(x_hbm, wqkv_hbm, wo_hbm, w1_hbm, w2_hbm, out_hbm,
            x_v, wqkv_v, wo_v, w1_v, w2_v, xn_v, qkv_a, qkv_b, kp_v, vp_v, o_v, out_v,
            sem_x, sem_q, sem_w, sem_o):
    x_w, wqkv_w = x_hbm.bitcast(U32), wqkv_hbm.bitcast(U32)

    def x_cp(i):
        r = pl.ds(pl.multiple_of(i * TW, TW), TW)
        return pltpu.make_async_copy(x_w.at[r], x_v.at[r], sem_x.at[i])

    def wq_cp(c):
        col = pl.ds(pl.multiple_of(c * CW, CW), CW)
        return pltpu.make_async_copy(wqkv_w.at[:, col], wqkv_v.at[:, col], sem_q.at[c])

    rest = [pltpu.make_async_copy(w.bitcast(U32), v, sem_w.at[n])
            for n, (w, v) in enumerate(((wo_hbm, wo_v), (w1_hbm, w1_v), (w2_hbm, w2_v)))]

    def out_cp(i, slot, half=None):
        r = pl.ds(pl.multiple_of(i * T, T), T)
        c = slice(None) if half is None else pl.ds(half * (D // 2), D // 2)
        return pltpu.make_async_copy(out_v.at[slot, :, c], out_hbm.at[r, c], sem_o.at[slot])

    def weight(w_v, cols=slice(None)):
        return pltpu.bitcast(w_v[:, cols], BF)

    def tile(ref, i):
        return ref.at[pl.ds(pl.multiple_of(i * TW, TW), TW)]

    x_cp(0).start()
    x_cp(1).start()
    wq_cp(0).start()
    wq_cp(1).start()
    kp_v[...] = jnp.zeros_like(kp_v)
    vp_v[...] = jnp.zeros_like(vp_v)

    x_cp(0).wait()
    _drain(_ln_steps(0, x_v, xn_v.at[0:TW], 64))
    x_cp(1).wait()
    _drain(_ln_steps(1, x_v, xn_v.at[TW:2 * TW], 64))

    def qkv01(c):
        xn = pltpu.bitcast(xn_v[0:2 * TW, :], BF)
        col = pl.ds(pl.multiple_of(c * CW, CW), CW)
        r = jnp.dot(xn, weight(wqkv_v, col), preferred_element_type=F32)
        qkv_a[:, col] = pltpu.bitcast(r.astype(BF), U32)

    def p0a(it, _):
        wq_cp(it).wait()
        wq_cp(2 * it + 2).start()
        wq_cp(2 * it + 3).start()

        @pl.when(it == 2)
        def _():
            x_cp(2).start()
        qkv01(it)
        return 0

    def p0b(it, _):
        for j in range(3):
            wq_cp(3 + 3 * it + j).wait()

        @pl.when(it == 0)
        def _():
            x_cp(2).wait()
            for j in range(8, 12):
                wq_cp(j).start()

        @pl.when(it == 1)
        def _():
            for i in range(3, NT):
                x_cp(i).start()

        @pl.when(it == 2)
        def _():
            for cp in rest:
                cp.start()
        for j in range(3):
            qkv01(3 + 3 * it + j)
        for r in range(0, 96, 16):
            r0 = pl.multiple_of(80 * it + r, 16)
            y = _ln(_rows(x_v, 2 * T + r0, 16)).astype(BF)
            xn_v[pl.ds(pl.multiple_of(2 * TW + r0 // 2, 8), 8), :] = pltpu.bitcast(y, U32)
        return 0

    jax.lax.fori_loop(0, 3, p0a, 0)
    jax.lax.fori_loop(0, 3, p0b, 0)

    def pstep(s, _):
        @pl.when(s + 3 < NT)
        def _():
            x_cp(s + 3).wait()
        xn = pltpu.bitcast(tile(xn_v, (s + 2) % 3)[...], BF)
        r = jnp.dot(xn, weight(wqkv_v), preferred_element_type=F32)
        tile(qkv_b, s)[...] = pltpu.bitcast(r.astype(BF), U32)
        _interleave(_ln_steps(jnp.minimum(s + 3, NT - 1), x_v, tile(xn_v, s % 3), 8),
                    _attention_steps(s * PJ, PJ, 2 * G, 0, qkv_a, kp_v, vp_v, o_v))
        return 0

    jax.lax.fori_loop(0, NT - 2, pstep, 0)
    for cp in rest:
        cp.wait()

    def estep(i, _):
        slot = i % 2

        @pl.when(i >= 2)
        def _():
            out_cp(i - 2, slot).wait()
        HT = T // 2
        hs = []
        for a in range(2):
            rw = pl.multiple_of(i * TW + a * (HT // 2), HT // 2)
            o = pltpu.bitcast(o_v[pl.ds(rw, HT // 2), :], BF)
            att = jnp.dot(o, weight(wo_v), preferred_element_type=F32).astype(BF).astype(F32)
            h = _rows(x_v, pl.multiple_of(i * T + a * HT, HT), HT) + att
            hs.append(h.astype(BF).astype(F32))
        hid = []
        for a in range(2):
            hn = jnp.concatenate([_ln(hs[a][r:r + 16]) for r in range(0, HT, 16)], axis=0).astype(BF)
            hid.append(jnp.maximum(jnp.dot(hn, weight(w1_v), preferred_element_type=F32), 0.0))
        hid = jnp.concatenate(hid, axis=0).astype(BF)
        h = jnp.concatenate(hs, axis=0)
        for a in range(2):
            cs = slice(a * (D // 2), (a + 1) * (D // 2))
            out = h[:, cs] + jnp.dot(hid, weight(w2_v, cs), preferred_element_type=F32)
            out_v[slot, :, cs] = out.astype(BF)
            out_cp(i, slot, a).start()
        _drain(_attention_steps(2 * G + i * EJ, EJ, NT * G, 2, qkv_b, kp_v, vp_v, o_v))
        return 0

    jax.lax.fori_loop(0, NT, estep, 0)
    out_cp(NT - 2, (NT - 2) % 2).wait()
    out_cp(NT - 1, (NT - 1) % 2).wait()


@jax.jit
def pallas_sequential_preLN__sliding_local_dilated__dense_activation_relu__prompt_kernel(
    A_x: jax.Array,
    A_wqkv: jax.Array,
    A_wo: jax.Array,
    B_x: jax.Array,
    B_w1: jax.Array,
    B_w2: jax.Array,
):
    del B_x
    out = pl.pallas_call(
        _kernel,
        out_shape=jax.ShapeDtypeStruct((S, D), BF),
        in_specs=[pl.BlockSpec(memory_space=pl.ANY)] * 5,
        out_specs=pl.BlockSpec(memory_space=pl.ANY),
        scratch_shapes=[
            pltpu.VMEM((S // 2, D), U32),
            pltpu.VMEM((D // 2, 3 * D), U32),
            pltpu.VMEM((D // 2, D), U32),
            pltpu.VMEM((D // 2, FF), U32),
            pltpu.VMEM((FF // 2, D), U32),
            pltpu.VMEM((3 * TW, D), U32),
            pltpu.VMEM((2 * TW, 3 * D), U32),
            pltpu.VMEM(((NT - 2) * TW, 3 * D), U32),
            pltpu.VMEM((G, 128, 128), U32),
            pltpu.VMEM((G, 128, 128), U32),
            pltpu.VMEM(((NT + 1) * TW, D), U32),
            pltpu.VMEM((2, T, D), BF),
            pltpu.SemaphoreType.DMA((NT,)),
            pltpu.SemaphoreType.DMA((3 * D // CW,)),
            pltpu.SemaphoreType.DMA((3,)),
            pltpu.SemaphoreType.DMA((2,)),
        ],
        compiler_params=pltpu.CompilerParams(vmem_limit_bytes=100 * 1024 * 1024),
        name="fused",
    )(A_x.reshape(S, D), A_wqkv, A_wo, B_w1, B_w2)
    return out.reshape(1, S, D)
```

```python
import jax
import jax.numpy as jnp
from jax.experimental import pallas as pl
from jax.experimental.pallas import tpu as pltpu

BF = jnp.bfloat16
F32 = jnp.float32
U32 = jnp.uint32
I32 = jnp.int32

S, D, FF = 2048, 1024, 3584
DH, W = 32, 8
EPS = 1e-5
SCALE = DH ** -0.5

T = 256
NT = S // T
TW = T // 2
G = D // 128
CW = 256
PJ = 3
EJ = 7


def _ln(x):
    m = jnp.mean(x, axis=-1, keepdims=True)
    xc = x - m
    v = jnp.mean(xc * xc, axis=-1, keepdims=True)
    return xc * jax.lax.rsqrt(v + EPS)


def _unpack(w, half):
    bits = (w << 16) if half == 0 else (w & jnp.uint32(0xFFFF0000))
    return jax.lax.bitcast_convert_type(bits, F32)


def _pack(lo, hi):
    lo = jax.lax.bitcast_convert_type(lo, U32) + jnp.uint32(0x8000)
    hi = jax.lax.bitcast_convert_type(hi, U32) + jnp.uint32(0x8000)
    return (lo >> 16) | (hi & jnp.uint32(0xFFFF0000))


def _sum_rows(p):
    sub = jax.lax.broadcasted_iota(I32, (8, 128), 0)

    def merge(a, b, sh):
        m = (sub & sh) == 0
        return jnp.where(m, a, b) + jnp.take_along_axis(jnp.where(m, b, a), sub ^ sh, axis=0)

    s1 = [merge(p[i], p[i + 4], 4) for i in range(4)]
    s2 = [merge(s1[i], s1[i + 2], 2) for i in range(2)]
    return merge(s2[0], s2[1], 1)


def _softmax_rows(part, valid):
    l = _sum_rows(part) * SCALE
    l = jnp.where(valid, l, -1e9)
    m = jnp.max(l, axis=0, keepdims=True)
    e = jnp.exp(l - m)
    a = e / jnp.sum(e, axis=0, keepdims=True)
    return [jnp.broadcast_to(a[w:w + 1], (8, 128)) for w in range(W)]


def _attention_steps(j0, nj, jend, tbase, qkv_ref, kp_ref, vp_ref, o_ref):
    lane8 = jax.lax.broadcasted_iota(I32, (8, 128), 1)
    sub8 = jax.lax.broadcasted_iota(I32, (8, 128), 0)
    never = (lane8 + j0) < 0

    def chain(x, dep):
        if dep is None:
            return x
        return jnp.where(never, jax.lax.bitcast_convert_type(dep, x.dtype), x)

    def job(n):
        j = j0 + n
        jc = jnp.minimum(j, jend - 1)
        return jc // G, jnp.where(j < jend, j // G, NT), jc % G

    def load_t(n, part):
        t, _, g = job(n)
        rows = pl.ds(pl.multiple_of((t - tbase) * TW, TW), TW)
        return qkv_ref[rows, pl.ds(pl.multiple_of((part * G + g) * 128, 128), 128)].T

    def store_t(n, words):
        _, slot, g = job(n)
        rows = pl.ds(pl.multiple_of(slot * TW, TW), TW)
        o_ref[rows, pl.ds(pl.multiple_of(g * 128, 128), 128)] = words.T

    def shifted(cur, prv, w):
        if w == 0:
            return cur
        return pltpu.roll(jnp.where(lane8 >= 128 - w, prv, cur), w, 1)

    q_nxt, k_nxt, v_nxt = load_t(0, 0), load_t(0, 1), load_t(0, 2)
    prev = None
    pend = None
    for n in range(nj):
        t, _, g = job(n)
        valid = (lane8 + t * TW) >= sub8
        qT, kT, vT = q_nxt, k_nxt, v_nxt
        kp = kp_ref[g]
        vp = vp_ref[g]
        kp_ref[g] = kT
        vp_ref[g] = vT
        words = []
        for h in range(4):
            sl = [slice(32 * h + 8 * j, 32 * h + 8 * j + 8) for j in range(4)]
            kws = [[shifted(kT[sl[j]], kp[sl[j]], w) for j in range(4)] for w in range(W)]
            att = []
            for half in range(2):
                q = [_unpack(qT[sl[j]], half) for j in range(4)]
                part = []
                for w in range(W):
                    k = [_unpack(kws[w][j], half) for j in range(4)]
                    k[0] = chain(k[0], prev)
                    prev = (q[0] * k[0] + q[1] * k[1]) + (q[2] * k[2] + q[3] * k[3])
                    part.append(prev)
                att.append(_softmax_rows(part, valid))
                prev = att[-1][0]
            for j in range(4):
                vw = [shifted(vT[sl[j]], vp[sl[j]], w) for w in range(W)]
                acc = []
                for half in range(2):
                    a = att[half][0] * chain(_unpack(vw[0], half), prev)
                    for w in range(1, W):
                        a = a + att[half][w] * _unpack(vw[w], half)
                    acc.append(a)
                    prev = a
                words.append(_pack(*acc))
            if h == 0 and pend is not None:
                store_t(n - 1, pend)
                pend = None
            if n + 1 < nj:
                if h == 1:
                    q_nxt = load_t(n + 1, 0)
                elif h == 2:
                    k_nxt = load_t(n + 1, 1)
                elif h == 3:
                    v_nxt = load_t(n + 1, 2)
            yield
        pend = jnp.concatenate(words, axis=0)
    store_t(nj - 1, pend)


def _rows(ref, r0, n):
    w = ref[pl.ds(pl.multiple_of(r0 // 2, n // 2), n // 2), :]
    return pltpu.bitcast(w, BF).astype(F32)


def _ln_steps(t, x_ref, xn_ref, rows):
    blk = max(rows, 16)
    for r in range(0, T, blk):
        x = _rows(x_ref, t * T + r, blk)
        ys = []
        for q in range(0, blk, rows):
            ys.append(_ln(x[q:q + rows]))
            if q + rows < blk:
                yield
        y = ys[0] if len(ys) == 1 else jnp.concatenate(ys, axis=0)
        xn_ref[r // 2:(r + blk) // 2, :] = pltpu.bitcast(y.astype(BF), U32)
        yield


def _drain(gen):
    for _ in gen:
        pass


def _interleave(*gens):
    alive = list(gens)
    while alive:
        for gen in list(alive):
            if next(gen, alive) is alive:
                alive.remove(gen)


def _kernel(x_hbm, wqkv_hbm, wo_hbm, w1_hbm, w2_hbm, out_hbm,
            x_v, wqkv_v, wo_v, w1_v, w2_v, xn_v, qkv_a, qkv_b, kp_v, vp_v, o_v, out_v,
            sem_x, sem_q, sem_w, sem_o):
    x_w, wqkv_w = x_hbm.bitcast(U32), wqkv_hbm.bitcast(U32)

    def x_cp(i):
        r = pl.ds(pl.multiple_of(i * TW, TW), TW)
        return pltpu.make_async_copy(x_w.at[r], x_v.at[r], sem_x.at[i])

    def wq_cp(c):
        col = pl.ds(pl.multiple_of(c * CW, CW), CW)
        return pltpu.make_async_copy(wqkv_w.at[:, col], wqkv_v.at[:, col], sem_q.at[c])

    rest = [pltpu.make_async_copy(w.bitcast(U32), v, sem_w.at[n])
            for n, (w, v) in enumerate(((wo_hbm, wo_v), (w1_hbm, w1_v), (w2_hbm, w2_v)))]

    def out_cp(i, slot, half=None):
        r = pl.ds(pl.multiple_of(i * T, T), T)
        c = slice(None) if half is None else pl.ds(half * (D // 2), D // 2)
        return pltpu.make_async_copy(out_v.at[slot, :, c], out_hbm.at[r, c], sem_o.at[slot])

    def weight(w_v, cols=slice(None)):
        return pltpu.bitcast(w_v[:, cols], BF)

    def tile(ref, i):
        return ref.at[pl.ds(pl.multiple_of(i * TW, TW), TW)]

    for cp in (x_cp(0), x_cp(1), wq_cp(0), wq_cp(1)):
        cp.start()
    kp_v[...] = jnp.zeros_like(kp_v)
    vp_v[...] = jnp.zeros_like(vp_v)

    x_cp(0).wait()
    _drain(_ln_steps(0, x_v, xn_v.at[0:TW], 64))
    x_cp(1).wait()
    wq_cp(0).wait()
    wq_cp(2).start()
    wq_cp(3).start()
    for t in range(2):
        if t == 1:
            _drain(_ln_steps(1, x_v, xn_v.at[TW:2 * TW], 8))
        xn = pltpu.bitcast(xn_v[t * TW:(t + 1) * TW, :], BF)
        r = jnp.dot(xn, weight(wqkv_v, slice(0, CW)), preferred_element_type=F32)
        qkv_a[t * TW:(t + 1) * TW, 0:CW] = pltpu.bitcast(r.astype(BF), U32)

    def qkv01(c):
        xn = pltpu.bitcast(xn_v[0:2 * TW, :], BF)
        col = pl.ds(pl.multiple_of(c * CW, CW), CW)
        r = jnp.dot(xn, weight(wqkv_v, col), preferred_element_type=F32)
        qkv_a[:, col] = pltpu.bitcast(r.astype(BF), U32)

    def p0a(it, _):
        wq_cp(it).wait()
        wq_cp(2 * it + 2).start()
        wq_cp(2 * it + 3).start()

        @pl.when(it == 1)
        def _():
            x_cp(2).start()
        qkv01(it)
        return 0

    def p0b(it, _):
        for j in range(3):
            wq_cp(3 + 3 * it + j).wait()

        @pl.when(it == 0)
        def _():
            x_cp(2).wait()
            for j in range(8, 12):
                wq_cp(j).start()

        @pl.when(it == 1)
        def _():
            for i in range(3, NT):
                x_cp(i).start()

        @pl.when(it == 2)
        def _():
            for cp in rest:
                cp.start()
        for j in range(3):
            qkv01(3 + 3 * it + j)
        for r in range(0, 96, 16):
            r0 = pl.multiple_of(80 * it + r, 16)
            y = _ln(_rows(x_v, 2 * T + r0, 16)).astype(BF)
            xn_v[pl.ds(pl.multiple_of(2 * TW + r0 // 2, 8), 8), :] = pltpu.bitcast(y, U32)
        return 0

    jax.lax.fori_loop(1, 3, p0a, 0)
    jax.lax.fori_loop(0, 3, p0b, 0)

    def pstep(s, _):
        @pl.when(s + 3 < NT)
        def _():
            x_cp(s + 3).wait()
        xn = pltpu.bitcast(tile(xn_v, (s + 2) % 3)[...], BF)
        r = jnp.dot(xn, weight(wqkv_v), preferred_element_type=F32)
        tile(qkv_b, s)[...] = pltpu.bitcast(r.astype(BF), U32)
        _interleave(_ln_steps(jnp.minimum(s + 3, NT - 1), x_v, tile(xn_v, s % 3), 8),
                    _attention_steps(s * PJ, PJ, 2 * G, 0, qkv_a, kp_v, vp_v, o_v))
        return 0

    jax.lax.fori_loop(0, NT - 2, pstep, 0)
    for cp in rest:
        cp.wait()

    def estep(i, _):
        slot = i % 2

        @pl.when(i >= 2)
        def _():
            out_cp(i - 2, slot).wait()
        HT = T // 2
        hs = []
        for a in range(2):
            rw = pl.multiple_of(i * TW + a * (HT // 2), HT // 2)
            o = pltpu.bitcast(o_v[pl.ds(rw, HT // 2), :], BF)
            att = jnp.dot(o, weight(wo_v), preferred_element_type=F32).astype(BF).astype(F32)
            h = _rows(x_v, pl.multiple_of(i * T + a * HT, HT), HT) + att
            hs.append(h.astype(BF).astype(F32))
        hid = []
        for a in range(2):
            hn = jnp.concatenate([_ln(hs[a][r:r + 16]) for r in range(0, HT, 16)], axis=0).astype(BF)
            hid.append(jnp.maximum(jnp.dot(hn, weight(w1_v), preferred_element_type=F32), 0.0))
        hid = jnp.concatenate(hid, axis=0).astype(BF)
        h = jnp.concatenate(hs, axis=0)
        for a in range(2):
            cs = slice(a * (D // 2), (a + 1) * (D // 2))
            out = h[:, cs] + jnp.dot(hid, weight(w2_v, cs), preferred_element_type=F32)
            out_v[slot, :, cs] = out.astype(BF)
            out_cp(i, slot, a).start()
        _drain(_attention_steps(2 * G + i * EJ, EJ, NT * G, 2, qkv_b, kp_v, vp_v, o_v))
        return 0

    jax.lax.fori_loop(0, NT, estep, 0)
    out_cp(NT - 2, (NT - 2) % 2).wait()
    out_cp(NT - 1, (NT - 1) % 2).wait()


@jax.jit
def pallas_sequential_preLN__sliding_local_dilated__dense_activation_relu__prompt_kernel(
    A_x: jax.Array,
    A_wqkv: jax.Array,
    A_wo: jax.Array,
    B_x: jax.Array,
    B_w1: jax.Array,
    B_w2: jax.Array,
):
    del B_x
    out = pl.pallas_call(
        _kernel,
        out_shape=jax.ShapeDtypeStruct((S, D), BF),
        in_specs=[pl.BlockSpec(memory_space=pl.ANY)] * 5,
        out_specs=pl.BlockSpec(memory_space=pl.ANY),
        scratch_shapes=[
            pltpu.VMEM((S // 2, D), U32),
            pltpu.VMEM((D // 2, 3 * D), U32),
            pltpu.VMEM((D // 2, D), U32),
            pltpu.VMEM((D // 2, FF), U32),
            pltpu.VMEM((FF // 2, D), U32),
            pltpu.VMEM((3 * TW, D), U32),
            pltpu.VMEM((2 * TW, 3 * D), U32),
            pltpu.VMEM(((NT - 2) * TW, 3 * D), U32),
            pltpu.VMEM((G, 128, 128), U32),
            pltpu.VMEM((G, 128, 128), U32),
            pltpu.VMEM(((NT + 1) * TW, D), U32),
            pltpu.VMEM((2, T, D), BF),
            pltpu.SemaphoreType.DMA((NT,)),
            pltpu.SemaphoreType.DMA((3 * D // CW,)),
            pltpu.SemaphoreType.DMA((3,)),
            pltpu.SemaphoreType.DMA((2,)),
        ],
        compiler_params=pltpu.CompilerParams(vmem_limit_bytes=100 * 1024 * 1024),
        name="fused",
    )(A_x.reshape(S, D), A_wqkv, A_wo, B_w1, B_w2)
    return out.reshape(1, S, D)
```

```python
import jax
import jax.numpy as jnp
from jax.experimental import pallas as pl
from jax.experimental.pallas import tpu as pltpu

BF = jnp.bfloat16
F32 = jnp.float32
U32 = jnp.uint32
I32 = jnp.int32

S, D, FF = 2048, 1024, 3584
DH, W = 32, 8
EPS = 1e-5
SCALE = DH ** -0.5

T = 256
NT = S // T
TW = T // 2
G = D // 128
CW = 256
PJ = 3
EJ = 7
NS = 8
assert (NT - 2) * PJ >= 2 * G and all(2 * G + EJ * (i + 1) >= G * (i + 2) for i in range(NT - 1))


def _ln(x):
    m = jnp.mean(x, axis=-1, keepdims=True)
    xc = x - m
    v = jnp.mean(xc * xc, axis=-1, keepdims=True)
    return xc * jax.lax.rsqrt(v + EPS)


def _unpack(w, half):
    bits = (w << 16) if half == 0 else (w & jnp.uint32(0xFFFF0000))
    return jax.lax.bitcast_convert_type(bits, F32)


def _pack(lo, hi):
    lo = jax.lax.bitcast_convert_type(lo, U32) + jnp.uint32(0x8000)
    hi = jax.lax.bitcast_convert_type(hi, U32) + jnp.uint32(0x8000)
    return (lo >> 16) | (hi & jnp.uint32(0xFFFF0000))


def _sum_rows(p):
    sub = jax.lax.broadcasted_iota(I32, (8, 128), 0)

    def merge(a, b, sh):
        m = (sub & sh) == 0
        return jnp.where(m, a, b) + jnp.take_along_axis(jnp.where(m, b, a), sub ^ sh, axis=0)

    s1 = [merge(p[i], p[i + 4], 4) for i in range(4)]
    s2 = [merge(s1[i], s1[i + 2], 2) for i in range(2)]
    return merge(s2[0], s2[1], 1)


def _softmax_rows(part, valid):
    l = _sum_rows(part) * SCALE
    l = jnp.where(valid, l, -1e9)
    m = jnp.max(l, axis=0, keepdims=True)
    e = jnp.exp(l - m)
    a = e / jnp.sum(e, axis=0, keepdims=True)
    return [jnp.broadcast_to(a[w:w + 1], (8, 128)) for w in range(W)]


def _attention_steps(j0, nj, jend, tbase, qkv_ref, kp_ref, vp_ref, o_ref):
    lane8 = jax.lax.broadcasted_iota(I32, (8, 128), 1)
    sub8 = jax.lax.broadcasted_iota(I32, (8, 128), 0)
    never = (lane8 + j0) < 0

    def chain(x, dep):
        if dep is None:
            return x
        return jnp.where(never, jax.lax.bitcast_convert_type(dep, x.dtype), x)

    def job(n):
        j = j0 + n
        jc = jnp.minimum(j, jend - 1)
        return jc // G, jnp.where(j < jend, j // G, NT), jc % G

    def load_t(n, part):
        t, _, g = job(n)
        rows = pl.ds(pl.multiple_of((t - tbase) * TW, TW), TW)
        return qkv_ref[rows, pl.ds(pl.multiple_of((part * G + g) * 128, 128), 128)].T

    def store_t(n, words):
        _, slot, g = job(n)
        rows = pl.ds(pl.multiple_of(slot * TW, TW), TW)
        o_ref[rows, pl.ds(pl.multiple_of(g * 128, 128), 128)] = words.T

    def shifted(cur, prv, w):
        if w == 0:
            return cur
        return pltpu.roll(jnp.where(lane8 >= 128 - w, prv, cur), w, 1)

    q_nxt, k_nxt, v_nxt = load_t(0, 0), load_t(0, 1), load_t(0, 2)
    prev = None
    pend = None
    for n in range(nj):
        t, _, g = job(n)
        valid = (lane8 + t * TW) >= sub8
        qT, kT, vT = q_nxt, k_nxt, v_nxt
        kp = kp_ref[g]
        vp = vp_ref[g]
        kp_ref[g] = kT
        vp_ref[g] = vT
        words = []
        for h in range(4):
            sl = [slice(32 * h + 8 * j, 32 * h + 8 * j + 8) for j in range(4)]
            kws = [[shifted(kT[sl[j]], kp[sl[j]], w) for j in range(4)] for w in range(W)]
            att = []
            for half in range(2):
                q = [_unpack(qT[sl[j]], half) for j in range(4)]
                part = []
                for w in range(W):
                    k = [_unpack(kws[w][j], half) for j in range(4)]
                    k[0] = chain(k[0], prev)
                    prev = (q[0] * k[0] + q[1] * k[1]) + (q[2] * k[2] + q[3] * k[3])
                    part.append(prev)
                att.append(_softmax_rows(part, valid))
                prev = att[-1][0]
            for j in range(4):
                vw = [shifted(vT[sl[j]], vp[sl[j]], w) for w in range(W)]
                acc = []
                for half in range(2):
                    a = att[half][0] * chain(_unpack(vw[0], half), prev)
                    for w in range(1, W):
                        a = a + att[half][w] * _unpack(vw[w], half)
                    acc.append(a)
                    prev = a
                words.append(_pack(*acc))
            if h == 0 and pend is not None:
                store_t(n - 1, pend)
                pend = None
            if n + 1 < nj:
                if h == 1:
                    q_nxt = load_t(n + 1, 0)
                elif h == 2:
                    k_nxt = load_t(n + 1, 1)
                elif h == 3:
                    v_nxt = load_t(n + 1, 2)
            yield
        pend = jnp.concatenate(words, axis=0)
    store_t(nj - 1, pend)


def _rows(ref, r0, n):
    w = ref[pl.ds(pl.multiple_of(r0 // 2, n // 2), n // 2), :]
    return pltpu.bitcast(w, BF).astype(F32)


def _ln_steps(t, x_ref, xn_ref, rows):
    blk = max(rows, 16)
    for r in range(0, T, blk):
        x = _rows(x_ref, t * T + r, blk)
        ys = []
        for q in range(0, blk, rows):
            ys.append(_ln(x[q:q + rows]))
            if q + rows < blk:
                yield
        y = ys[0] if len(ys) == 1 else jnp.concatenate(ys, axis=0)
        xn_ref[r // 2:(r + blk) // 2, :] = pltpu.bitcast(y.astype(BF), U32)
        yield


def _drain(gen):
    for _ in gen:
        pass


def _interleave(*gens):
    alive = list(gens)
    while alive:
        for gen in list(alive):
            if next(gen, alive) is alive:
                alive.remove(gen)


def _kernel(x_hbm, wqkv_hbm, wo_hbm, w1_hbm, w2_hbm, out_hbm,
            x_v, wqkv_v, wo_v, w1_v, w2_v, xn_v, qkv_a, qkv_b, kp_v, vp_v, o_v, out_v,
            sem_x, sem_q, sem_w, sem_o):
    x_w, wqkv_w = x_hbm.bitcast(U32), wqkv_hbm.bitcast(U32)

    def x_cp(i):
        r = pl.ds(pl.multiple_of(i * TW, TW), TW)
        return pltpu.make_async_copy(x_w.at[r], x_v.at[r], sem_x.at[i])

    def wq_cp(c):
        col = pl.ds(pl.multiple_of(c * CW, CW), CW)
        return pltpu.make_async_copy(wqkv_w.at[:, col], wqkv_v.at[:, col], sem_q.at[c])

    rest = [pltpu.make_async_copy(w.bitcast(U32), v, sem_w.at[n])
            for n, (w, v) in enumerate(((wo_hbm, wo_v), (w1_hbm, w1_v), (w2_hbm, w2_v)))]

    def out_cp(i, slot, part=None):
        r = pl.ds(pl.multiple_of(i * T, T), T)
        c = slice(None) if part is None else pl.ds(part * (D // NS), D // NS)
        return pltpu.make_async_copy(out_v.at[slot, :, c], out_hbm.at[r, c], sem_o.at[slot])

    def weight(w_v, cols=slice(None)):
        return pltpu.bitcast(w_v[:, cols], BF)

    def tile(ref, i):
        return ref.at[pl.ds(pl.multiple_of(i * TW, TW), TW)]

    for cp in (x_cp(0), x_cp(1), wq_cp(0), wq_cp(1)):
        cp.start()
    kp_v[...] = jnp.zeros_like(kp_v)
    vp_v[...] = jnp.zeros_like(vp_v)

    x_cp(0).wait()
    _drain(_ln_steps(0, x_v, xn_v.at[0:TW], 64))
    x_cp(1).wait()
    wq_cp(0).wait()
    wq_cp(2).start()
    wq_cp(3).start()
    for t in range(2):
        if t == 1:
            _drain(_ln_steps(1, x_v, xn_v.at[TW:2 * TW], 8))
        xn = pltpu.bitcast(xn_v[t * TW:(t + 1) * TW, :], BF)
        r = jnp.dot(xn, weight(wqkv_v, slice(0, CW)), preferred_element_type=F32)
        qkv_a[t * TW:(t + 1) * TW, 0:CW] = pltpu.bitcast(r.astype(BF), U32)

    def qkv01(c):
        xn = pltpu.bitcast(xn_v[0:2 * TW, :], BF)
        col = pl.ds(pl.multiple_of(c * CW, CW), CW)
        r = jnp.dot(xn, weight(wqkv_v, col), preferred_element_type=F32)
        qkv_a[:, col] = pltpu.bitcast(r.astype(BF), U32)

    def p0a(it, _):
        wq_cp(it).wait()
        wq_cp(2 * it + 2).start()
        wq_cp(2 * it + 3).start()

        @pl.when(it == 1)
        def _():
            x_cp(2).start()
        qkv01(it)
        return 0

    def p0b(it, _):
        for j in range(3):
            wq_cp(3 + 3 * it + j).wait()
        for j in range(3):
            qkv01(3 + 3 * it + j)
        for r in range(0, 96, 16):
            r0 = pl.multiple_of(80 * it + r, 16)
            y = _ln(_rows(x_v, 2 * T + r0, 16)).astype(BF)
            xn_v[pl.ds(pl.multiple_of(2 * TW + r0 // 2, 8), 8), :] = pltpu.bitcast(y, U32)
        return 0

    jax.lax.fori_loop(1, 3, p0a, 0)
    for c in range(8, 3 * D // CW):
        wq_cp(c).start()
    for i in range(3, NT):
        x_cp(i).start()
    x_cp(2).wait()
    jax.lax.fori_loop(0, 3, p0b, 0)
    for cp in rest:
        cp.start()

    def pstep(s, _):
        @pl.when(s + 3 < NT)
        def _():
            x_cp(s + 3).wait()
        xn = pltpu.bitcast(tile(xn_v, (s + 2) % 3)[...], BF)
        r = jnp.dot(xn, weight(wqkv_v), preferred_element_type=F32)
        tile(qkv_b, s)[...] = pltpu.bitcast(r.astype(BF), U32)
        _interleave(_ln_steps(jnp.minimum(s + 3, NT - 1), x_v, tile(xn_v, s % 3), 8),
                    _attention_steps(s * PJ, PJ, 2 * G, 0, qkv_a, kp_v, vp_v, o_v))
        return 0

    jax.lax.fori_loop(0, NT - 2, pstep, 0)
    for cp in rest:
        cp.wait()

    def estep(i, _):
        slot = i % 2

        @pl.when(i >= 2)
        def _():
            out_cp(i - 2, slot).wait()
        HT = T // 2
        hs = []
        for a in range(2):
            rw = pl.multiple_of(i * TW + a * (HT // 2), HT // 2)
            o = pltpu.bitcast(o_v[pl.ds(rw, HT // 2), :], BF)
            att = jnp.dot(o, weight(wo_v), preferred_element_type=F32).astype(BF).astype(F32)
            h = _rows(x_v, pl.multiple_of(i * T + a * HT, HT), HT) + att
            hs.append(h.astype(BF).astype(F32))
        hid = []
        for a in range(2):
            hn = jnp.concatenate([_ln(hs[a][r:r + 16]) for r in range(0, HT, 16)], axis=0).astype(BF)
            hid.append(jnp.maximum(jnp.dot(hn, weight(w1_v), preferred_element_type=F32), 0.0))
        hid = jnp.concatenate(hid, axis=0).astype(BF)
        h = jnp.concatenate(hs, axis=0)
        for a in range(NS):
            cs = slice(a * (D // NS), (a + 1) * (D // NS))
            out = h[:, cs] + jnp.dot(hid, weight(w2_v, cs), preferred_element_type=F32)
            out_v[slot, :, cs] = out.astype(BF)
            out_cp(i, slot, a).start()
        _drain(_attention_steps(2 * G + i * EJ, EJ, NT * G, 2, qkv_b, kp_v, vp_v, o_v))
        return 0

    jax.lax.fori_loop(0, NT, estep, 0)
    out_cp(NT - 2, (NT - 2) % 2).wait()
    out_cp(NT - 1, (NT - 1) % 2).wait()


@jax.jit
def pallas_sequential_preLN__sliding_local_dilated__dense_activation_relu__prompt_kernel(
    A_x: jax.Array,
    A_wqkv: jax.Array,
    A_wo: jax.Array,
    B_x: jax.Array,
    B_w1: jax.Array,
    B_w2: jax.Array,
):
    del B_x
    out = pl.pallas_call(
        _kernel,
        out_shape=jax.ShapeDtypeStruct((S, D), BF),
        in_specs=[pl.BlockSpec(memory_space=pl.ANY)] * 5,
        out_specs=pl.BlockSpec(memory_space=pl.ANY),
        scratch_shapes=[
            pltpu.VMEM((S // 2, D), U32),
            pltpu.VMEM((D // 2, 3 * D), U32),
            pltpu.VMEM((D // 2, D), U32),
            pltpu.VMEM((D // 2, FF), U32),
            pltpu.VMEM((FF // 2, D), U32),
            pltpu.VMEM((3 * TW, D), U32),
            pltpu.VMEM((2 * TW, 3 * D), U32),
            pltpu.VMEM(((NT - 2) * TW, 3 * D), U32),
            pltpu.VMEM((G, 128, 128), U32),
            pltpu.VMEM((G, 128, 128), U32),
            pltpu.VMEM(((NT + 1) * TW, D), U32),
            pltpu.VMEM((2, T, D), BF),
            pltpu.SemaphoreType.DMA((NT,)),
            pltpu.SemaphoreType.DMA((3 * D // CW,)),
            pltpu.SemaphoreType.DMA((3,)),
            pltpu.SemaphoreType.DMA((2,)),
        ],
        compiler_params=pltpu.CompilerParams(vmem_limit_bytes=100 * 1024 * 1024),
        name="fused",
    )(A_x.reshape(S, D), A_wqkv, A_wo, B_w1, B_w2)
    return out.reshape(1, S, D)
```
